```python
import os as _os
_os.environ.setdefault("JAX_PLATFORMS", "cpu")
import jax
import jax.numpy as jnp

def _softmax(x, axis=-1):
    return jax.nn.softmax(x, axis=axis)
def _gelu(x):
    return jax.nn.gelu(x, approximate=True)
def _silu(x):
    return jax.nn.silu(x)
def _sigmoid(x):
    return jax.nn.sigmoid(x)
def _layernorm(x, axis=-1, eps=1e-5):
    m = jnp.mean(x, axis=axis, keepdims=True)
    v = jnp.var(x, axis=axis, keepdims=True)
    return (x - m) / jnp.sqrt(v + eps)
def _scatter_add(tgt, idx, src, axis=0):
    return tgt.at[idx].add(src)
def _segment_sum(src, seg, n):
    return jax.ops.segment_sum(src, seg, n)
class _Rng:
    def __init__(self, key):
        self._k = key
    def _next(self):
        self._k, sub = jax.random.split(self._k)
        return sub
    def normal(self, shape):
        return jax.random.normal(self._next(), shape, dtype=jnp.bfloat16)
    def randint(self, lo, hi, shape):
        return jax.random.randint(self._next(), shape, lo, hi, dtype=jnp.int32)
    def uniform(self, shape, lo=0.0, hi=1.0):
        return jax.random.uniform(self._next(), shape, jnp.bfloat16, lo, hi)
    def permutation(self, n):
        return jax.random.permutation(self._next(), n)


kernel_name = 'standalone__layernorm_linear__sampling'

def setup_inputs():
    _rng = _Rng(jax.random.key(int.from_bytes(__import__("os").urandom(4), "little")))
    _w = (lambda a: (lambda t: t.astype(jnp.bfloat16) if jnp.issubdtype(t.dtype, jnp.floating) else t)(jnp.asarray(a)))
    B, S, D = 1024, 32, 576
    return {
        "x": _w((lambda *s: _rng.normal(s) * 0.05)(B, S, D)),
        "g": _w((lambda *s: _rng.normal(s) * 0.05)(D) + 1.0),
        "b": _w((lambda *s: _rng.normal(s) * 0.05)(D)),
        "w": _w((lambda *s: _rng.normal(s) * 0.05)(D, D)),
    }

def reference(x, g, b, w):
    return (_layernorm(x, axis=-1) * g + b) @ w
```

```python
import functools
import jax, jax.numpy as jnp, numpy as np
from jax import lax
from jax.experimental import pallas as pl
from jax.experimental.pallas import tpu as pltpu

D = 576
H = 288
Q = 144
S = 32
L = 1024
f32, bf16, u32 = jnp.float32, jnp.bfloat16, jnp.uint32

def pk(v): return pltpu.bitcast(v.astype(bf16), u32)
def upk(v): return pltpu.bitcast(v, bf16)
def tile(v, n): return jnp.concatenate([v] * (n // 8), axis=0) if n > 8 else v
cat = lambda *a: jnp.concatenate(a, axis=0)
dot = functools.partial(jnp.dot, preferred_element_type=f32)

def make(hold=15, dma=True, U=1, every=4, lo=0.0, hi=0.9, merge=True, prenorm=True, fwd=False, rev=True, flo=0.8, flags=None):
    NR = D // 8
    def red(xb, s, l0, fn, pins=None, link=None):
        acc = None
        for i in range(NR):
            t = fn(xb[s, pl.ds(8 * i, 8), pl.ds(l0, 256)].astype(f32))
            acc = t if acc is None else acc + t
            if link is not None and i % every == 0: acc = link(i / NR, acc)
            if pins is not None and i % every == every - 1: pins.append((i / NR, acc[:, :128])); pins.append((i / NR, acc[:, 128:]))
        return jnp.broadcast_to(jnp.sum(acc, axis=0, keepdims=True) * (1.0 / D), (8, 256))
    def mean_pass(xb, s, l0, pins=None, link=None): return red(xb, s, l0, lambda t: t, pins, link)
    def var_pass(xb, s, l0, m, pins=None, link=None): return lax.rsqrt(red(xb, s, l0, lambda t: jnp.square(t - m), pins, link) + 1e-5)
    def norm(xb, s, l0, m, r, pins=None, link=None):
        ys = []
        for i in range(NR):
            if link is not None and i % every == 0: m = link(i / NR, m)
            y = (xb[s, pl.ds(8 * i, 8), pl.ds(l0, 256)].astype(f32) - m) * r
            ys.append(y)
            if pins is not None: pins.append((i / NR, y[:, :128])); pins.append((i / NR, y[:, 128:]))
        return cat(*ys)

    def mm(y, wl, d_ref):
        a1, b1, a2, b2, ea, eb = y[:256, :128], y[:256, 128:], y[256:512, :128], y[256:512, 128:], y[512:, :128], y[512:, 128:]
        F = {1: a1 - b2, 2: a1, 3: b1 - b2, 4: a2 - a1, 5: b2, 6: a1 - b1, 7: a2 - b2}
        E = {3: eb, 4: ea, 6: eb, 7: ea}
        W = lambda i, j: upk(wl[2 * (i - 1) + j])
        Wh = lambda i, j, h: upk(wl[2 * (i - 1) + j, pl.ds(h * Q // 2, Q // 2), :])
        P = {i: dot(upk(wl[14 + n // 2, pl.ds((n % 2) * Q // 2, Q // 2), :]), cat(E[i], F[i][192:]).astype(bf16)) for n, i in enumerate((3, 4, 6, 7))}
        def second(i, h): return (cat(F[i][128:192], E[i]) if (h == 1 and i in E) else F[i][128:]).astype(bf16)
        def init(i, u):
            if i in E: return cat(P[i], P[i]) + u
            if i == 5: return d_ref[pl.ds(0, H), :] + u
            if i == 2: return d_ref[pl.ds(H, H), :] + u
            return u
        def pair(i, k):
            if merge:
                u = dot(W(i, 0), F[i][:128].astype(bf16)); v = dot(W(i, 1), F[i][128:].astype(bf16))
                p = dot(W(k, 0), F[k][:128].astype(bf16)); q = cat(dot(Wh(k, 1, 0), second(k, 0)), dot(Wh(k, 1, 1), second(k, 1)))
            else:
                r = [[dot(Wh(i, 0, h), F[i][:128].astype(bf16)), dot(Wh(i, 1, h), second(i, h)), dot(Wh(k, 0, h), F[k][:128].astype(bf16)), dot(Wh(k, 1, h), second(k, h))] for h in range(2)]
                u, v, p, q = [cat(r[0][n], r[1][n]) for n in range(4)]
            return init(i, u) + v, init(k, p) + q
        m2, m4 = pair(2, 4)
        c21 = m2 + m4
        n5, n3 = pair(5, 3)
        c12 = n5 + n3; c11 = m4 + n5; c22 = m2 + n3
        m1, m7 = pair(1, 7)
        c11 = (c11 + m1) + m7; c22 = c22 - m1
        r = [[dot(Wh(6, 0, h), F[6][:128].astype(bf16)), dot(Wh(6, 1, h), second(6, h))] for h in range(2)]
        c22 = c22 + (init(6, cat(r[0][0], r[1][0])) + cat(r[0][1], r[1][1]))
        rows = lambda c: [c[8 * i:8 * i + 8] for i in range(c.shape[0] // 8)]
        return (c21, c12, c11, c22), rows(P[3]) + rows(m4) + rows(n3) + rows(m7) + rows(r[1][1])

    def kern(x_hbm, g_hbm, b_hbm, w_hbm, o_hbm, xb, ob, g_ref, b_ref, w_ref, wl, d_ref, yb, isem, osem):
        def rd(s): return pltpu.make_async_copy(x_hbm.at[s], xb.at[s], isem.at[s])
        small = [pltpu.make_async_copy(a, b, isem.at[S]) for a, b in ((g_hbm, g_ref), (b_hbm, b_ref), (w_hbm, w_ref))]
        for c in small: c.start()
        if dma:
            for s in range(S): rd(s).start()
        else:
            cp = pltpu.make_async_copy(x_hbm.at[0, pl.ds(0, 16)], xb.at[0, pl.ds(0, 16)], isem.at[0]); cp.start(); cp.wait()
        for c in small: c.wait()
        g = g_ref[...].astype(f32).reshape(1, D)
        b = b_ref[...].astype(f32).reshape(1, D)
        T = [w_ref[pl.ds(128 * k, 128), :].astype(f32).T for k in range(4)]
        we = w_ref[pl.ds(512, 64), :].astype(f32)
        T.append(cat(we, we).T)
        lane = lax.broadcasted_iota(jnp.int32, (Q, 128), 1) < 64
        ge = jnp.concatenate([g[:, 512:], g[:, 512:]], axis=1)
        be = jnp.concatenate([b[:, 512:], jnp.zeros((1, 64), f32)], axis=1)
        db = T[4] * be
        for k in range(4): db = db + T[k] * b[:, 128 * k:128 * (k + 1)]
        d_ref[...] = jnp.broadcast_to(jnp.sum(db, axis=1, keepdims=True), (D, 128))
        T = [T[k] * g[:, 128 * k:128 * (k + 1)] for k in range(4)] + [T[4] * ge]
        A = lambda i, j: [T[2 * (j - 1) + c][H * (i - 1):H * i] for c in range(2)]
        add = lambda p, q: [u + v for u, v in zip(p, q)]
        sub = lambda p, q: [u - v for u, v in zip(p, q)]
        V = {1: add(A(1, 1), A(2, 2)), 2: add(A(2, 1), A(2, 2)), 3: A(1, 1), 4: A(2, 2), 5: add(A(1, 1), A(1, 2)),
             6: sub(A(1, 1), A(2, 1)), 7: sub(A(1, 2), A(2, 2))}
        e1, e2 = T[4][:H], T[4][H:]
        VE = {3: e1, 4: e2, 6: e2 - e1, 7: e1 - e2}
        for i in range(1, 8):
            v0, v1 = V[i]
            if i in VE:
                t1, b1 = v1[:Q], v1[Q:]
                et, eb = VE[i][:Q], VE[i][Q:]
                n = (3, 4, 6, 7).index(i)
                wl[14 + n // 2, pl.ds((n % 2) * Q // 2, Q // 2), :] = pk(jnp.where(lane, et, b1))
                v1 = cat(jnp.where(lane, t1, t1 - b1), jnp.where(lane, b1, eb - et))
            wl[2 * (i - 1)] = pk(v0); wl[2 * (i - 1) + 1] = pk(v1)
        if dma: rd(0).wait()
        m0 = mean_pass(xb, 0, 0); r0 = var_pass(xb, 0, 0, m0); m1 = mean_pass(xb, 0, 256)
        if prenorm:
            yb[...] = norm(xb, 0, 0, m0, r0)
            r1 = var_pass(xb, 0, 256, m1); m2 = mean_pass(xb, 0, 512)
            m0, r0, m1 = m1, r1, m2
        def body(i, c):
            m0, r0, m1 = c
            if dma:
                for u in range(U):
                    @pl.when(i * U + u + 1 < S)
                    def _(): rd(jnp.minimum(i * U + u + 1, S - 1)).wait()
            never = i < 0
            pos = lambda j: (jnp.minimum(i * U + j // 4, S - 1), 256 * (j % 4))
            if prenorm: y = yb[...]
            for j in range(4 * U):
                pins = []
                k = j + int(prenorm)
                if not prenorm: y = norm(xb, *pos(k), m0, r0)
                cs, ticks = mm(y, wl, d_ref)
                last = j == 4 * U - 1
                def link(fr, v):
                    tk = ticks[int(fr * flo * len(ticks))]
                    return jnp.where(never, jnp.concatenate([tk, tk], axis=1), v)
                lk = link if (fwd or last) else None
                pn = pins if (rev and not last) else None
                if prenorm: y = norm(xb, *pos(k), m0, r0, pn, lk)
                r1 = var_pass(xb, *pos(k + 1), m1, pn, lk)
                m2 = mean_pass(xb, *pos(k + 2), pn, lk)
                m0, r0, m1 = m1, r1, m2
                cs = [[c[8 * n:8 * n + 8] for n in range(H // 8)] for c in cs]
                slots = [(0, n) for n in range(36)] + [(1, n) for n in range(36)] + [(2, n) for n in range(36)] + [(3, n) for n in range(18)]
                for fr, v in pins:
                    a, n = slots[int((lo + fr * (hi - lo)) * len(slots))]
                    cs[a][n] = jnp.where(never, v, cs[a][n])
                s, l0 = pos(j)
                for c, (half, ln) in zip(cs, ((1, 0), (0, 1), (0, 0), (1, 1))):
                    ob[s, pl.ds(H * half, H), pl.ds(l0 + 128 * ln, 128)] = cat(*c).astype(bf16)
            if prenorm: yb[...] = y
            if dma:
                h = hold // U
                @pl.when(i == h)
                def _(): pltpu.make_async_copy(ob.at[pl.ds(0, (h + 1) * U)], o_hbm.at[pl.ds(0, (h + 1) * U)], osem).start()
                @pl.when(i > h)
                def _(): pltpu.make_async_copy(ob.at[pl.ds(i * U, U)], o_hbm.at[pl.ds(i * U, U)], osem).start()
            return m0, r0, m1
        lax.fori_loop(0, S // U, body, (m0, r0, m1))
        if dma: pltpu.make_async_copy(ob, o_hbm, osem).wait()
        else:
            cp = pltpu.make_async_copy(ob.at[0, pl.ds(0, 16)], o_hbm.at[0, pl.ds(0, 16)], osem); cp.start(); cp.wait()

    @jax.jit
    def f(x, g, b, w):
        xt = jnp.transpose(x, (1, 2, 0))
        an = pl.BlockSpec(memory_space=pl.ANY)
        o = pl.pallas_call(kern,
            in_specs=[an, an, an, an], out_specs=an,
            out_shape=jax.ShapeDtypeStruct((S, D, L), bf16),
            scratch_shapes=[pltpu.VMEM((S, D, L), bf16), pltpu.VMEM((S, D, L), bf16),
                            pltpu.VMEM((D,), bf16), pltpu.VMEM((D,), bf16), pltpu.VMEM((D, D), bf16),
                            pltpu.VMEM((16, H // 2, 128), u32), pltpu.VMEM((D, 128), f32), pltpu.VMEM((D, 256), f32),
                            pltpu.SemaphoreType.DMA((S + 1,)), pltpu.SemaphoreType.DMA(())],
            compiler_params=pltpu.CompilerParams(vmem_limit_bytes=110*2**20, flags=flags),
            name="v6")(xt, g, b, w)
        return jnp.transpose(o, (2, 0, 1))
    return f


_impl = make(merge=False, prenorm=True, fwd=True, U=2, hold=15)


@jax.jit
def pallas_standalone__layernorm_linear__sampling_kernel(x, g, b, w):
    return _impl(x, g, b, w)
```

```python
import functools

import jax
import jax.numpy as jnp
from jax import lax
from jax.experimental import pallas as pl
from jax.experimental.pallas import tpu as pltpu

f32, bf16, u32 = jnp.float32, jnp.bfloat16, jnp.uint32

EPS = 1e-5
S, D, L = 32, 576, 1024
HALF, QUARTER = D // 2, D // 4
UNIT = 512

SPLIT = (2, 5)
WHOLE = (1, 3, 4, 6, 7)
EXTRA = {3: 1, 4: 0, 6: 1, 7: 0}
BIAS_ROW = {5: 0, 2: HALF}

HEAD = (1, 1, 2, 4)
LOOP_UNITS, LOOP_STEPS = 8, 7
QUEUE_ROUNDS = (1, 5, 8, 12)
FIRST_WRITE = 123

COST_MEAN, COST_VAR, COST_EXTRA, COST_WHOLE, COST_SPLIT = 20, 34, 56, 42, 24
SUM_WEIGHT, LEAD_ROUNDS = 1.3, 2

_W_TILE = {
    key: n
    for n, key in enumerate(
        [("shared", i) for i in EXTRA]
        + [(i, t, h) for i in WHOLE for t in range(2) for h in range(2)]
        + [("split", i, k) for i in SPLIT for k in range(1, 8)]
    )
}


def _block_rows():
    sizes = (
        [((p, "extra", t), 64) for p in range(2) for t in range(2)]
        + [((p, i), 256) for p in range(2) for i in WHOLE]
        + [(("split", i, k), 128) for i in SPLIT for k in range(1, 8)]
    )
    start, total = {}, 0
    for key, n in sizes:
        start[key] = total
        total += n
    return start, total


_X_ROW, _X_ROWS = _block_rows()


def _cat(*parts):
    return jnp.concatenate(parts, axis=0)


def _vregs(v):
    return [v[r : r + 8] for r in range(0, v.shape[0], 8)]


def _w_forms(w11, w12, w21, w22):
    return {1: w11 + w22, 2: w21 + w22, 3: w11, 4: w22, 5: w11 + w12, 6: w11 - w21, 7: w12 - w22}


def _x_forms(a1, b1, a2, b2):
    return {1: a1 - b2, 2: a1, 3: b1 - b2, 4: a2 - a1, 5: b2, 6: a1 - b1, 7: a2 - b2}


def _build_weights(wt_ref, g_ref, b_ref, tiles_ref, bias_ref):
    g = g_ref[...].astype(f32).reshape(1, D)
    b = b_ref[...].astype(f32).reshape(1, D)
    gs = [g[:, k : k + 128] for k in range(0, 512, 128)]
    bs = [b[:, k : k + 128] for k in range(0, 512, 128)]
    gs.append(jnp.concatenate([g[:, 512:], g[:, 512:]], axis=1))
    bs.append(jnp.concatenate([b[:, 512:], jnp.zeros((1, 64), f32)], axis=1))
    low = lax.broadcasted_iota(jnp.int32, (16, 128), 1) < 64
    for r in range(0, QUARTER, 16):
        wg = {}
        for q in range(4):
            w = [wt_ref[c, pl.ds(QUARTER * q + r, 16), :].astype(f32) for c in range(5)]
            wb = functools.reduce(lambda u, v: u + v, [w[c] * bs[c] for c in range(5)])
            wb = jnp.sum(wb, axis=1, keepdims=True)
            bias_ref[pl.ds(QUARTER * q + r, 16), :] = jnp.broadcast_to(wb, (16, 128))
            for c in range(5):
                wg[q, c] = w[c] * gs[c]

        def put(key, v, r=r):
            tiles_ref[_W_TILE[key], pl.ds(r, 16), :] = v.astype(bf16)

        v = {
            (t, h): _w_forms(wg[h, t], wg[h, 2 + t], wg[2 + h, t], wg[2 + h, 2 + t])
            for t in range(2)
            for h in range(2)
        }
        ve = [
            {3: e1, 4: e2, 6: e2 - e1, 7: e1 - e2}
            for e1, e2 in ((wg[0, 4], wg[2, 4]), (wg[1, 4], wg[3, 4]))
        ]
        for i in EXTRA:
            up, lo = v[1, 0][i], v[1, 1][i]
            put(("shared", i), jnp.where(low, ve[0][i], lo))
            v[1, 0][i] = jnp.where(low, up, up - lo)
            v[1, 1][i] = jnp.where(low, lo, ve[1][i] - ve[0][i])
        for i in WHOLE:
            for (t, h), forms in v.items():
                put((i, t, h), forms[i])
        for i in SPLIT:
            for k, form in _w_forms(v[0, 0][i], v[1, 0][i], v[0, 1][i], v[1, 1][i]).items():
                put(("split", i, k), form)


def _normalize(x_ref, slab, lane, blocks_ref):
    def load(k, row, rows, p):
        return x_ref[slab[k], pl.ds(row, rows), pl.ds(lane + 256 * p, 256)].astype(f32)

    def feature_mean(k, fn, cost):
        out = []
        for p in range(2):
            acc = None
            for row in range(0, D, 32):
                hold = yield cost
                for r in range(row, row + 32, 8):
                    term = fn(load(k, r, 8, p), p)
                    acc = term if acc is None else acc + term
                    acc = hold(acc) if r == row else acc
                yield [acc[:, :128], acc[:, 128:]]
            total = jnp.sum(acc, axis=0, keepdims=True)
            mean = total * (1.0 / D)
            mean = mean + ((total - 512.0 * mean) - 64.0 * mean) * (1.0 / D)
            out.append(jnp.broadcast_to(mean, (8, 256)))
        return out

    mean = yield from feature_mean(0, lambda x, p: x, COST_MEAN)
    var = yield from feature_mean(1, lambda x, p: jnp.square(x - mean[p]), COST_VAR)
    scale = [lax.rsqrt(v + EPS) for v in var]

    def xhat(row, p):
        y = (load(2, row, 16, p) - _cat(mean[p], mean[p])) * _cat(scale[p], scale[p])
        return y[:, :128], y[:, 128:]

    def put(key, row, v):
        blocks_ref[pl.ds(_X_ROW[key] + row, 16), :] = v.astype(bf16)

    for p in range(2):
        hold = yield COST_EXTRA
        mean[p] = hold(mean[p])
        for row in range(0, 64, 16):
            for t, v in enumerate(xhat(512 + row, p)):
                put((p, "extra", t), row, v)
        yield None
    for row in range(0, 128, 16):
        forms = {}
        for p in range(2):
            for c in range(2):
                hold = yield COST_WHOLE
                mean[p] = hold(mean[p])
                forms[p, c] = _x_forms(*xhat(128 * c + row, p), *xhat(256 + 128 * c + row, p))
                for i in WHOLE:
                    put((p, i), 128 * c + row, forms[p, c][i])
                yield None
        for i in SPLIT:
            yield COST_SPLIT
            split = _x_forms(forms[0, 0][i], forms[1, 0][i], forms[0, 1][i], forms[1, 1][i])
            for k, v in split.items():
                put(("split", i, k), row, v)
            yield None


def _rounds(units):
    seq, first = [], []
    for j in range(units):
        first.append(-(-len(seq) // 4))
        if len(seq) % 4 == 0:
            shared = (3, 4, 6, 7)
            order = ((4, 0), (3, 0), (4, 1), (3, 1), (1, 0), (6, 0), (1, 1), (6, 1), (7, 0), (7, 1))
        else:
            shared = (4, 7, 3, 6)
            order = ((4, 0), (4, 1), (3, 0), (3, 1), (7, 0), (1, 0), (6, 0), (1, 1), (6, 1), (7, 1))
        seq += [(j, ("split", i, k)) for i in SPLIT for k in (4, 3, 1, 6, 5, 7, 2)]
        for p in range(2):
            seq += [(j, (p, "shared", i)) for i in shared]
            seq += [(j, (p, i, t, h)) for i, h in order for t in range(2)]
    return [seq[r : r + 4] for r in range(0, len(seq), 4)], first


def _product(res, bias_ref, p, i, h):
    def once(key, fn):
        if key not in res:
            res[key] = fn()
        return res[key]

    if i in WHOLE:
        if i in EXTRA:
            return once((p, i, h), lambda: (res[p, "shared", i] + res[p, i, 0, h]) + res[p, i, 1, h])
        return once((p, i, h), lambda: res[p, i, 0, h] + res[p, i, 1, h])

    def m(k):
        return res["split", i, k]

    def biased(k, row):
        return once(("bias", i, k), lambda: bias_ref[pl.ds(BIAS_ROW[i] + row, QUARTER), :] + m(k))

    return once(
        (p, i, h),
        {
            (0, 0): lambda: ((m(1) + m(4)) + biased(5, 0)) + m(7),
            (1, 0): lambda: biased(5, 0) + m(3),
            (0, 1): lambda: biased(2, QUARTER) + m(4),
            (1, 1): lambda: biased(2, QUARTER) + ((m(3) - m(1)) + m(6)),
        }[p, h],
    )


def _output(res, bias_ref, p, half, h):
    def m(i):
        return _product(res, bias_ref, p, i, h)

    if half == 0:
        return ((m(5) + m(4)) + m(1)) + m(7), m(5) + m(3)
    return m(2) + m(4), (m(2) + m(3)) + (m(6) - m(1))


def _pace(rounds, first):
    sums = [0] * (len(rounds) + 1)

    class Result:
        def __init__(self, r):
            self.r = r

        def __add__(self, other):
            r = max(self.r, other.r)
            sums[r + 1] += QUARTER // 8
            return Result(r)

        __sub__ = __add__

        def __getitem__(self, _):
            return self

    res = [{} for _ in first]
    for r, passes in enumerate(rounds):
        for j, key in passes:
            res[j][key] = Result(r)
    for unit in res:
        for p, half, h in ((p, half, h) for p in range(2) for half in range(2) for h in range(2)):
            a, b = _output(unit, Result(0), p, half, h)
            _ = (a + a, b + b)
    total = 36 * (COST_MEAN + COST_VAR) + 2 * COST_EXTRA + 32 * COST_WHOLE + 16 * COST_SPLIT
    edges = [LEAD_ROUNDS if len(first) == 1 else 0]
    edges += [r - LEAD_ROUNDS for r in first[1:]] + [len(rounds)]
    pace = {}
    for j in range(len(first)):
        span = range(edges[j], edges[j + 1])
        level = (total + SUM_WEIGHT * sum(sums[r] for r in span)) / len(span)
        done = 0.0
        for r in span:
            pace[r] = (j, done, level - SUM_WEIGHT * sums[r])
            done += pace[r][2]
    return pace


def _kernel(
    x_hbm, g_hbm, b_hbm, w_hbm, o_hbm,
    x_ref, o_ref, blocks0, blocks1, bias_ref, w_ref, wt_ref, tiles_ref, g_ref, b_ref,
    zero_ref, sems,
):
    blocks = (blocks0, blocks1)
    words = [ref.bitcast(u32) for ref in blocks]
    tile_words = tiles_ref.bitcast(u32)
    for k in range(4):
        zero_ref[k] = 0

    def read(index, sem):
        return pltpu.make_async_copy(x_hbm.at[index], x_ref.at[index], sems.at[sem])

    def write(first, count, row, rows, lane, lanes):
        index = (pl.ds(first, count), pl.ds(row, rows), pl.ds(lane, lanes))
        pltpu.make_async_copy(o_ref.at[index], o_hbm.at[index], sems.at[0]).start()

    def read_unit(u, sem):
        return read((u // 2, slice(None), pl.ds(UNIT * (u % 2), UNIT)), sem)

    def read_step(i, slabs):
        return read(pl.ds(4 * i + 5, slabs), 6 + len(HEAD) + i)

    w_reads = [
        pltpu.make_async_copy(w_hbm.at[rows], w_ref.at[rows], sems.at[1 + k])
        for k, rows in enumerate((pl.ds(0, 256), pl.ds(256, 256), pl.ds(512, 64)))
    ]
    gb_reads = [
        pltpu.make_async_copy(g_hbm, g_ref, sems.at[4]),
        pltpu.make_async_copy(b_hbm, b_ref, sems.at[4]),
    ]
    head_first = [sum(HEAD[:k]) for k in range(len(HEAD))]
    head_reads = [
        [read_unit(u + 1, 6 + k) for u in range(head_first[k], head_first[k] + HEAD[k])]
        for k in range(len(HEAD))
    ]
    head_reads[-1].append(read_unit(sum(HEAD) + 1, 5 + len(HEAD)))
    first_read = read_unit(0, 5)
    for copy in w_reads + gb_reads + [first_read] + sum(head_reads, []):
        copy.start()
    for i in range(LOOP_STEPS):
        read_step(i, 4 if i < LOOP_STEPS - 1 else 3).start()

    for k in range(2):
        w_reads[k].wait()
        for c in range(2 * k, 2 * k + 2):
            wt_ref[c] = w_ref[pl.ds(128 * c, 128), :].T
    for copy in [w_reads[2]] + gb_reads:
        copy.wait()
    last_rows = w_ref[pl.ds(512, 64), :]
    wt_ref[4] = _cat(last_rows, last_rows).T
    _build_weights(wt_ref, g_ref, b_ref, tiles_ref, bias_ref)
    first_read.wait()
    steps = _normalize(x_ref, [zero_ref[k] for k in (1, 2, 3)], 0, blocks[0])
    for _ in steps:
        steps.send(lambda v: v)

    def queue_writes(i, j, q, pending):
        assert all(unit >= j for unit, *_ in pending)

        def piece(first, n):
            for k in range(9 * n // 2, 9 * (n + 1) // 2):
                write(first, 4, 8 * k, 8, 0, L)

        t = 4 * (sum(HEAD) + j) + q - FIRST_WRITE
        group = 4 * i + t // 8
        assert FIRST_WRITE + 8 * 13 >= 16 * 14
        pl.when((group >= 0) & (group < 14))(lambda: piece(4 * jnp.clip(group, 0, 13), t % 8))

        @pl.when(i == LOOP_STEPS - 1)
        def _():
            if j in (4, 5):
                piece(56, 4 * (j - 4) + q)
            if j == 6:
                for k in range(9 * q, 9 * q + 9):
                    write(60, 2, 8 * k, 8, 0, L)
            if j == 7 and q == 0:
                for half in range(2):
                    write(62 + half, 1, 0, HALF, 0, UNIT)
            if j == 7 and q == 3:
                assert all(p == 1 for _, p, *_ in pending)
                for half in range(2):
                    write(62 + half, 1, 0, HALF, UNIT, 256)

    def segment(u0, units, i=None):
        def place(j):
            slab = (u0 + j) // 2
            if i is not None:
                slab = jnp.minimum(slab + (LOOP_UNITS // 2) * i, S - 1)
            return slab, UNIT * ((u0 + j) % 2)

        zero = zero_ref[0]
        never = zero != 0
        zeros = [zero_ref[k] for k in (1, 2, 3)]

        def x_words(j, key, row, rows):
            start = pl.multiple_of(zero + (_X_ROW[key] + row) // 2, 8)
            return words[(u0 + j) % 2][pl.ds(start, rows // 2), :]

        def right(j, key):
            if key[0] == "split":
                return x_words(j, key, 0, 128)
            p, i_ = key[0], key[2] if key[1] == "shared" else key[1]
            if key[1] == "shared":
                return _cat(x_words(j, (p, "extra", EXTRA[i_]), 0, 64), x_words(j, (p, i_), 192, 64))
            if key[2:] == (1, 1) and i_ in EXTRA:
                return _cat(x_words(j, (p, i_), 128, 64), x_words(j, (p, "extra", EXTRA[i_]), 0, 64))
            return x_words(j, (p, i_), 128 * key[2], 128)

        rounds, first = _rounds(units)
        pace = _pace(rounds, first)
        steps = []
        for j in range(units):
            slab, lane = place(j + 1)
            steps.append(_normalize(x_ref, [slab + z for z in zeros], lane, blocks[(u0 + j + 1) % 2]))
        cost = [next(s) for s in steps]
        spent = [0] * units
        res = [{} for _ in range(units)]
        popped = []
        pending = [
            (j, p, half, h)
            for j in range(units) for p in range(2) for h in range(2) for half in range(2)
        ]
        for r, passes in enumerate(rounds):
            rhs = [right(j, key) for j, key in passes]
            lhs = [
                _vregs(tile_words[_W_TILE[key if key[0] == "split" else key[1:]]])
                for _, key in passes
            ]
            for e in range(len(lhs[0]) if r in pace else 0):
                j, before, during = pace[r]
                due = before + during * (e + 1) / len(lhs[0]) + 1e-6
                ran = []
                while cost[j] is not None and spent[j] + cost[j] <= due:
                    hold = lambda v: v
                    if j == units - 1:
                        tick = popped[r - LEAD_ROUNDS][2 * e]
                        hold = functools.partial(jnp.where, never, jnp.concatenate([tick, tick], axis=1))
                    partial = steps[j].send(hold)
                    if j < units - 1 and partial:
                        ran = [pltpu.bitcast(v, u32) for v in partial]
                    elif j < units - 1:
                        ran = [x_words(j + 1, (0, "extra", 0), 0, 16)]
                    spent[j] += cost[j]
                    cost[j] = next(steps[j], None)
                for n, v in enumerate(ran):
                    lhs[n][e] = jnp.where(never, v, lhs[n][e])
            for (j, key), a, b in zip(passes, lhs, rhs):
                res[j][key] = y = jnp.dot(
                    pltpu.bitcast(_cat(*a), bf16), pltpu.bitcast(b, bf16), preferred_element_type=f32
                )
            popped.append(_vregs(y))
            for j in range(units):
                if i is not None and r - first[j] in QUEUE_ROUNDS:
                    queue_writes(i, j, QUEUE_ROUNDS.index(r - first[j]), pending)
            for j, p, half, h in list(pending):
                if all((p, k, 1, h) in res[j] for k in ((1, 3, 4, 7), (1, 3, 4, 6))[half]):
                    slab, lane = place(j)
                    y = jnp.concatenate(_output(res[j], bias_ref, p, half, h), axis=1)
                    rows, lanes = pl.ds(QUARTER * h, QUARTER), pl.ds(lane + 256 * p, 256)
                    o_ref[2 * slab + half, rows, lanes] = y.astype(bf16)
                    pending.remove((j, p, half, h))
        assert not pending and all(c is None for c in cost)

    for k, units in enumerate(HEAD):
        for copy in head_reads[k]:
            copy.wait()
        segment(head_first[k], units)

    def loop_step(i, _):
        pl.when(i < LOOP_STEPS - 1)(lambda: read_step(jnp.minimum(i, LOOP_STEPS - 2), 4).wait())
        pl.when(i == LOOP_STEPS - 1)(lambda: read_step(LOOP_STEPS - 1, 3).wait())
        segment(sum(HEAD), LOOP_UNITS, i)

    lax.fori_loop(0, LOOP_STEPS, loop_step, None)
    for half in range(2):
        write(62 + half, 1, 0, HALF, L - 256, 256)
    pltpu.make_async_copy(o_ref, o_hbm, sems.at[0]).wait()


@jax.jit
def pallas_standalone__layernorm_linear__sampling_kernel(
    x: jax.Array,
    g: jax.Array,
    b: jax.Array,
    w: jax.Array,
):
    assert x.shape == (L, S, D) and w.shape == (D, D)
    hbm = pl.BlockSpec(memory_space=pl.ANY)
    out = pl.pallas_call(
        _kernel,
        in_specs=[hbm] * 4,
        out_specs=hbm,
        out_shape=jax.ShapeDtypeStruct((2 * S, HALF, L), bf16),
        scratch_shapes=[
            pltpu.VMEM((S, D, L), bf16),
            pltpu.VMEM((2 * S, HALF, L), bf16),
            pltpu.VMEM((_X_ROWS, 128), bf16),
            pltpu.VMEM((_X_ROWS, 128), bf16),
            pltpu.VMEM((D, 128), f32),
            pltpu.VMEM((D, D), bf16),
            pltpu.VMEM((5, D, 128), bf16),
            pltpu.VMEM((-(-len(_W_TILE) // 4) * 4, QUARTER, 128), bf16),
            pltpu.VMEM((D,), bf16),
            pltpu.VMEM((D,), bf16),
            pltpu.SMEM((4,), jnp.int32),
            pltpu.SemaphoreType.DMA((6 + len(HEAD) + LOOP_STEPS,)),
        ],
        compiler_params=pltpu.CompilerParams(
            vmem_limit_bytes=110 * 2**20,
            disable_bounds_checks=True,
            disable_semaphore_checks=True,
        ),
        name="layernorm_linear",
    )(jnp.transpose(x, (1, 2, 0)), g, b, w)
    return jnp.transpose(out.reshape(S, D, L), (2, 0, 1))
```

```python
import functools

import jax
import jax.numpy as jnp
from jax import lax
from jax.experimental import pallas as pl
from jax.experimental.pallas import tpu as pltpu

f32, bf16, u32 = jnp.float32, jnp.bfloat16, jnp.uint32

EPS = 1e-5
S, D, L = 32, 576, 1024
HALF, THIRD, QUARTER = D // 2, D // 3, D // 4
UNIT = 512

SPLIT = (2, 5)
WHOLE = (1, 3, 4, 6, 7)
EXTRA = {3: 1, 4: 0, 6: 1, 7: 0}
BIAS_ROW = {5: 0, 2: HALF}

HEAD = (1, 1, 2, 4)
LOOP_UNITS, EARLY_STEPS, LOOP_STEPS = 8, 4, 7
LATE_SLAB = (sum(HEAD) + LOOP_UNITS * EARLY_STEPS) // 2

PACED_SLAB, PACED_UNIT = 25, 9
PACED_ROUNDS = (0, 1, 2, 4, 5, 6, 8, 9, 10, 12, 13, 14)

QUEUE_ROUNDS = (1, 5, 8, 12)
FIRST_WRITE = 122
LAST_DELAY = 2
LAST_ROUND = 90

COST_MEAN, COST_VAR, COST_EXTRA, COST_WHOLE, COST_SPLIT = 20, 34, 56, 42, 24
SUM_WEIGHT, LEAD_ROUNDS = 1.0, 2

_W_TILE = {
    key: n
    for n, key in enumerate(
        [("shared", i) for i in EXTRA]
        + [(i, t, h) for i in WHOLE for t in range(2) for h in range(2)]
        + [("split", i, k) for i in SPLIT for k in range(1, 8)]
    )
}


def _block_rows():
    sizes = (
        [((p, "extra", t), 64) for p in range(2) for t in range(2)]
        + [((p, i), 256) for p in range(2) for i in WHOLE]
        + [(("split", i, k), 128) for i in SPLIT for k in range(1, 8)]
    )
    start, total = {}, 0
    for key, n in sizes:
        start[key] = total
        total += n
    return start, total


_X_ROW, _X_ROWS = _block_rows()


def _cat(*parts):
    return jnp.concatenate(parts, axis=0)


def _vregs(v):
    return [v[r : r + 8] for r in range(0, v.shape[0], 8)]


def _dot(a, b):
    return jnp.dot(pltpu.bitcast(a, bf16), pltpu.bitcast(b, bf16), preferred_element_type=f32)


def _w_forms(w11, w12, w21, w22):
    return {1: w11 + w22, 2: w21 + w22, 3: w11, 4: w22, 5: w11 + w12, 6: w11 - w21, 7: w12 - w22}


def _x_forms(a1, b1, a2, b2):
    return {1: a1 - b2, 2: a1, 3: b1 - b2, 4: a2 - a1, 5: b2, 6: a1 - b1, 7: a2 - b2}


def _build_weights(wt_ref, g_ref, b_ref, tiles_ref, bias_ref):
    g = g_ref[...].astype(f32).reshape(1, D)
    b = b_ref[...].astype(f32).reshape(1, D)
    gs = [g[:, k : k + 128] for k in range(0, 512, 128)]
    bs = [b[:, k : k + 128] for k in range(0, 512, 128)]
    gs.append(jnp.concatenate([g[:, 512:], g[:, 512:]], axis=1))
    bs.append(jnp.concatenate([b[:, 512:], jnp.zeros((1, 64), f32)], axis=1))
    low = lax.broadcasted_iota(jnp.int32, (16, 128), 1) < 64
    for r in range(0, QUARTER, 16):
        wg = {}
        for q in range(4):
            w = [wt_ref[c, pl.ds(QUARTER * q + r, 16), :].astype(f32) for c in range(5)]
            wb = functools.reduce(lambda u, v: u + v, [w[c] * bs[c] for c in range(5)])
            wb = jnp.sum(wb, axis=1, keepdims=True)
            bias_ref[pl.ds(QUARTER * q + r, 16), :] = jnp.broadcast_to(wb, (16, 128))
            for c in range(5):
                wg[q, c] = w[c] * gs[c]

        def put(key, v, r=r):
            tiles_ref[_W_TILE[key], pl.ds(r, 16), :] = v.astype(bf16)

        v = {
            (t, h): _w_forms(wg[h, t], wg[h, 2 + t], wg[2 + h, t], wg[2 + h, 2 + t])
            for t in range(2)
            for h in range(2)
        }
        ve = [
            {3: e1, 4: e2, 6: e2 - e1, 7: e1 - e2}
            for e1, e2 in ((wg[0, 4], wg[2, 4]), (wg[1, 4], wg[3, 4]))
        ]
        for i in EXTRA:
            up, lo = v[1, 0][i], v[1, 1][i]
            put(("shared", i), jnp.where(low, ve[0][i], lo))
            v[1, 0][i] = jnp.where(low, up, up - lo)
            v[1, 1][i] = jnp.where(low, lo, ve[1][i] - ve[0][i])
        for i in WHOLE:
            for (t, h), forms in v.items():
                put((i, t, h), forms[i])
        for i in SPLIT:
            for k, form in _w_forms(v[0, 0][i], v[1, 0][i], v[0, 1][i], v[1, 1][i]).items():
                put(("split", i, k), form)


def _normalize(x_ref, slab, lane, blocks_ref):
    def load(k, row, rows, p):
        index = (3 * slab[k] + row // THIRD, pl.ds(row % THIRD, rows), pl.ds(lane + 256 * p, 256))
        return x_ref[index].astype(f32)

    def feature_mean(k, fn, cost):
        out = []
        for p in range(2):
            acc = None
            for row in range(0, D, 32):
                hold = yield cost
                for r in range(row, row + 32, 8):
                    term = fn(load(k, r, 8, p), p)
                    acc = term if acc is None else acc + term
                    acc = hold(acc) if r == row else acc
                yield [acc[:, :128], acc[:, 128:]]
            total = jnp.sum(acc, axis=0, keepdims=True)
            mean = total * (1.0 / D)
            mean = mean + ((total - 512.0 * mean) - 64.0 * mean) * (1.0 / D)
            out.append(jnp.broadcast_to(mean, (8, 256)))
        return out

    mean = yield from feature_mean(0, lambda x, p: x, COST_MEAN)
    var = yield from feature_mean(1, lambda x, p: jnp.square(x - mean[p]), COST_VAR)
    scale = [lax.rsqrt(v + EPS) for v in var]

    def xhat(row, p):
        y = (load(2, row, 16, p) - _cat(mean[p], mean[p])) * _cat(scale[p], scale[p])
        return y[:, :128], y[:, 128:]

    def put(key, row, v):
        blocks_ref[pl.ds(_X_ROW[key] + row, 16), :] = v.astype(bf16)

    for p in range(2):
        hold = yield COST_EXTRA
        mean[p] = hold(mean[p])
        for row in range(0, 64, 16):
            for t, v in enumerate(xhat(512 + row, p)):
                put((p, "extra", t), row, v)
        yield None
    for row in range(0, 128, 16):
        forms = {}
        for p in range(2):
            for c in range(2):
                hold = yield COST_WHOLE
                mean[p] = hold(mean[p])
                forms[p, c] = _x_forms(*xhat(128 * c + row, p), *xhat(256 + 128 * c + row, p))
                for i in WHOLE:
                    put((p, i), 128 * c + row, forms[p, c][i])
                yield None
        for i in SPLIT:
            yield COST_SPLIT
            split = _x_forms(forms[0, 0][i], forms[1, 0][i], forms[0, 1][i], forms[1, 1][i])
            for k, v in split.items():
                put(("split", i, k), row, v)
            yield None


def _rounds(units):
    seq, first = [], []
    for j in range(units):
        first.append(-(-len(seq) // 4))
        if len(seq) % 4 == 0:
            shared = (3, 4, 6, 7)
            order = ((4, 0), (3, 0), (4, 1), (3, 1), (1, 0), (6, 0), (1, 1), (6, 1), (7, 0), (7, 1))
        else:
            shared = (4, 7, 3, 6)
            order = ((4, 0), (4, 1), (3, 0), (3, 1), (7, 0), (1, 0), (6, 0), (1, 1), (6, 1), (7, 1))
        seq += [(j, ("split", i, k)) for i in SPLIT for k in (4, 3, 1, 6, 5, 7, 2)]
        for p in range(2):
            seq += [(j, (p, "shared", i)) for i in shared]
            seq += [(j, (p, i, t, h)) for i, h in order for t in range(2)]
    return [seq[r : r + 4] for r in range(0, len(seq), 4)], first


def _product(res, bias_ref, p, i, h):
    def once(key, fn):
        if key not in res:
            res[key] = fn()
        return res[key]

    if i in WHOLE:
        u, v = res[p, i, 0, h], res[p, i, 1, h]
        if i not in EXTRA:
            return once((p, i, h), lambda: u + v)
        shared = res[p, "shared", i]
        return once((p, i, h), lambda: (shared + u) + v if i < 5 else shared + (u + v))

    def m(k):
        return res["split", i, k]

    def biased(k, row):
        return once(("bias", i, k), lambda: bias_ref[pl.ds(BIAS_ROW[i] + row, QUARTER), :] + m(k))

    return once(
        (p, i, h),
        {
            (0, 0): lambda: (m(1) + m(4)) + (biased(5, 0) + m(7)),
            (1, 0): lambda: biased(5, 0) + m(3),
            (0, 1): lambda: biased(2, QUARTER) + m(4),
            (1, 1): lambda: biased(2, QUARTER) + (m(3) + (m(6) - m(1))),
        }[p, h],
    )


def _output(res, bias_ref, p, half, h):
    def m(i):
        return _product(res, bias_ref, p, i, h)

    if half == 0:
        return (m(5) + m(4)) + (m(1) + m(7)), m(5) + m(3)
    return m(2) + m(4), (m(2) + m(3)) + (m(6) - m(1))


def _pace(rounds, first):
    sums = [0] * (len(rounds) + 1)

    class Result:
        def __init__(self, r):
            self.r = r

        def __add__(self, other):
            r = max(self.r, other.r)
            sums[r + 1] += QUARTER // 8
            return Result(r)

        __sub__ = __add__

        def __getitem__(self, _):
            return self

    res = [{} for _ in first]
    for r, passes in enumerate(rounds):
        for j, key in passes:
            res[j][key] = Result(r)
    for unit in res:
        for p, half, h in ((p, half, h) for p in range(2) for half in range(2) for h in range(2)):
            a, b = _output(unit, Result(0), p, half, h)
            _ = (a + a, b + b)
    total = 36 * (COST_MEAN + COST_VAR) + 2 * COST_EXTRA + 32 * COST_WHOLE + 16 * COST_SPLIT
    edges = [LEAD_ROUNDS if len(first) == 1 else 0]
    edges += [r - LEAD_ROUNDS for r in first[1:]] + [len(rounds)]
    pace = {}
    for j in range(len(first)):
        span = range(edges[j], edges[j + 1])
        level = (total + SUM_WEIGHT * sum(sums[r] for r in span)) / len(span)
        done = 0.0
        for r in span:
            pace[r] = (j, done, level - SUM_WEIGHT * sums[r])
            done += pace[r][2]
    return pace


def _kernel(
    x_hbm, g_hbm, b_hbm, w_hbm, o_hbm,
    x_ref, late_ref, o_ref, blocks0, blocks1, bias_ref, w_ref, wt_ref, tiles_ref, g_ref, b_ref,
    zero_ref, sems,
):
    blocks = (blocks0, blocks1)
    words = [ref.bitcast(u32) for ref in blocks]
    tile_words = tiles_ref.bitcast(u32)
    for k in range(4):
        zero_ref[k] = 0

    def read(slab, slabs, sem, lanes=slice(None), late=False):
        dst, base = (late_ref, LATE_SLAB) if late else (x_ref, 0)
        return pltpu.make_async_copy(
            x_hbm.at[pl.ds(3 * slab, 3 * slabs), :, lanes],
            dst.at[pl.ds(3 * (slab - base), 3 * slabs), :, lanes],
            sems.at[sem],
        )

    def write(first, count, row, rows, lane, lanes):
        index = (pl.ds(first, count), pl.ds(row, rows), pl.ds(lane, lanes))
        pltpu.make_async_copy(o_ref.at[index], o_hbm.at[index], sems.at[0]).start()

    w_reads = [
        pltpu.make_async_copy(w_hbm.at[rows], w_ref.at[rows], sems.at[1 + k])
        for k, rows in enumerate((pl.ds(0, 256), pl.ds(256, 256), pl.ds(512, 64)))
    ]
    gb_reads = [
        pltpu.make_async_copy(g_hbm, g_ref, sems.at[4]),
        pltpu.make_async_copy(b_hbm, b_ref, sems.at[4]),
    ]
    lower, upper = pl.ds(0, UNIT), pl.ds(UNIT, UNIT)
    first_read = read(0, 1, 5, lower)
    head_reads = [read(0, 1, 6, upper), read(1, 1, 7), read(2, 1, 8), read(3, 2, 9)]
    step_reads = [[read(4 * i + 5, 4, 10 + i)] for i in range(EARLY_STEPS - 1)]
    step_reads.append([read(LATE_SLAB - 3, 3, 13), read(LATE_SLAB, 1, 13, lower)])
    late_reads = [
        read(LATE_SLAB, 1, 14, upper, late=True),
        read(LATE_SLAB + 1, PACED_SLAB - LATE_SLAB - 1, 14, late=True),
    ]
    for copy in w_reads + gb_reads + [first_read] + head_reads:
        copy.start()
    for copy in sum(step_reads, []) + late_reads:
        copy.start(priority=1)
    step_reads[-1] += late_reads + [read(PACED_SLAB, S - PACED_SLAB, 15, late=True)]

    for k in range(2):
        w_reads[k].wait()
        for c in range(2 * k, 2 * k + 2):
            wt_ref[c] = w_ref[pl.ds(128 * c, 128), :].T
    for copy in [w_reads[2]] + gb_reads:
        copy.wait()
    last_rows = w_ref[pl.ds(512, 64), :]
    wt_ref[4] = _cat(last_rows, last_rows).T
    _build_weights(wt_ref, g_ref, b_ref, tiles_ref, bias_ref)
    first_read.wait()
    steps = _normalize(x_ref, [zero_ref[k] for k in (1, 2, 3)], 0, blocks[0])
    for _ in steps:
        steps.send(lambda v: v)

    def queue_writes(i, j, q, pending, late):
        assert all(unit >= j for unit, *_ in pending)
        t = 4 * (sum(HEAD) + j) + q - FIRST_WRITE
        if not late and t % 32 < 12:

            @pl.when(i == -(t // 32))
            def _():
                for k in range(3 * (t % 32), 3 * (t % 32) + 3):
                    write(0, 6, 8 * k, 8, 0, L)

        group, n = 4 * i + (t - 12) // 8, (t - 12) % 8
        assert all(FIRST_WRITE + 12 + 8 * k + LAST_DELAY * (k == 12) >= 8 * (2 * k + 5) for k in range(13))

        def pair(first, n):
            for k in range(9 * n // 2, 9 * (n + 1) // 2):
                write(first, 4, 8 * k, 8, 0, L)

        pl.when((group >= 0) & (group < 12))(lambda: pair(4 * jnp.clip(group, 0, 11) + 6, n))
        if late:

            @pl.when(i == LOOP_STEPS - 1)
            def _():
                m = t + 32 * (LOOP_STEPS - 1) - 12 - 8 * 12 - LAST_DELAY
                if 0 <= m < 8:
                    pair(54, m)
                elif 8 <= m < 12:
                    assert j >= 4
                    for k in range(9 * (m - 8), 9 * (m - 7)):
                        write(58, 2, 8 * k, 8, 0, L)

    def queue_last_writes(i, pending, left):
        for n, half, hs in list(left):
            if all((n // 2, n % 2, half, h) not in pending for h in hs):
                left.remove((n, half, hs))
                first, lane = 56 + 2 * (n // 4) + half, 256 * (n % 4)
                copy = functools.partial(write, first, 1, QUARTER * hs[0], QUARTER * len(hs), lane, 256)
                pl.when(i == LOOP_STEPS - 1)(copy)

    def queue_read(i, j, k, result):
        late_ref[3 * (S - LATE_SLAB), pl.ds(0, 16), pl.ds(0, 128)] = result.astype(bf16)
        n, count = LOOP_UNITS * i + sum(HEAD) + j - PACED_UNIT, 3 * (S - PACED_SLAB)

        @pl.when((n >= 0) & (n < count))
        def _():
            third = 3 * PACED_SLAB + jnp.clip(n, 0, count - 1)
            rows = pl.ds(k * THIRD // len(PACED_ROUNDS), THIRD // len(PACED_ROUNDS))
            dst = late_ref.at[third - 3 * LATE_SLAB, rows]
            pltpu.make_async_copy(x_hbm.at[third, rows], dst, sems.at[15]).start()

    def segment(u0, units, i=None, late=False):
        def place(j):
            slab = (u0 + j) // 2
            if i is not None:
                slab = jnp.minimum(slab + (LOOP_UNITS // 2) * i, S - 1)
            return slab, UNIT * ((u0 + j) % 2)

        zero = zero_ref[0]
        never = zero != 0
        zeros = [zero_ref[k] for k in (1, 2, 3)]

        def x_words(j, key, row, rows):
            start = pl.multiple_of(zero + (_X_ROW[key] + row) // 2, 8)
            return words[(u0 + j) % 2][pl.ds(start, rows // 2), :]

        def right(j, key):
            if key[0] == "split":
                return x_words(j, key, 0, 128)
            if key[1] == "shared":
                p, _, k = key
                return _cat(x_words(j, (p, "extra", EXTRA[k]), 0, 64), x_words(j, (p, k), 192, 64))
            p, k, t, h = key
            if (t, h) == (1, 1) and k in EXTRA:
                return _cat(x_words(j, (p, k), 128, 64), x_words(j, (p, "extra", EXTRA[k]), 0, 64))
            return x_words(j, (p, k), 128 * t, 128)

        rounds, first = _rounds(units)
        pace = _pace(rounds, first)
        steps = []
        for j in range(units):
            slab, lane = place(j + 1)
            src, slab = (late_ref, slab - LATE_SLAB) if late else (x_ref, slab)
            steps.append(_normalize(src, [slab + z for z in zeros], lane, blocks[(u0 + j + 1) % 2]))
        cost = [next(s) for s in steps]
        spent = [0] * units
        res = [{} for _ in range(units)]
        popped = []
        pending = [
            (j, p, half, h)
            for j in range(units) for p in range(2) for h in range(2) for half in range(2)
        ]
        left = [(n, half, (0, 1)) for n in range(8, 15) for half in range(2)]
        left += [(15, half, (h,)) for h in range(2) for half in range(2)]
        for r, passes in enumerate(rounds):
            rhs = [right(j, key) for j, key in passes]
            lhs = [
                _vregs(tile_words[_W_TILE[key if key[0] == "split" else key[1:]]])
                for _, key in passes
            ]
            for e in range(len(lhs[0]) if r in pace else 0):
                j, before, during = pace[r]
                due = before + during * (e + 1) / len(lhs[0]) + 1e-6
                ran = []
                while cost[j] is not None and spent[j] + cost[j] <= due:
                    hold = lambda v: v
                    if j == units - 1:
                        tick = popped[r - LEAD_ROUNDS][2 * e]
                        hold = functools.partial(jnp.where, never, jnp.concatenate([tick, tick], axis=1))
                    partial = steps[j].send(hold)
                    if j < units - 1 and partial:
                        ran = [pltpu.bitcast(v, u32) for v in partial]
                    elif j < units - 1:
                        ran = [x_words(j + 1, (0, "extra", 0), 0, 16)]
                    spent[j] += cost[j]
                    cost[j] = next(steps[j], None)
                for n, v in enumerate(ran):
                    lhs[n][e] = jnp.where(never, v, lhs[n][e])
            for (j, key), a, b in zip(passes, lhs, rhs):
                if len(passes) == 4:
                    res[j][key] = y = _dot(_cat(*a), b)
                else:
                    res[j][key] = y = _cat(_dot(_cat(*a[:5]), b), _dot(_cat(*a[5:]), b))
            popped.append(_vregs(y))
            for j in range(units):
                if i is not None and r - first[j] in QUEUE_ROUNDS:
                    queue_writes(i, j, QUEUE_ROUNDS.index(r - first[j]), pending, late)
                if i is not None and not late and r - first[j] in PACED_ROUNDS:
                    queue_read(i, j, PACED_ROUNDS.index(r - first[j]), y[:16])
            if late and r >= LAST_ROUND:
                queue_last_writes(i, pending, left)
            for j, p, half, h in list(pending):
                if all((p, k, 1, h) in res[j] for k in ((1, 3, 4, 7), (1, 3, 4, 6))[half]):
                    slab, lane = place(j)
                    y = jnp.concatenate(_output(res[j], bias_ref, p, half, h), axis=1)
                    rows, lanes = pl.ds(QUARTER * h, QUARTER), pl.ds(lane + 256 * p, 256)
                    o_ref[2 * slab + half, rows, lanes] = y.astype(bf16)
                    pending.remove((j, p, half, h))
        assert not pending and all(c is None for c in cost)
        if late:
            queue_last_writes(i, pending, left)

    for k, units in enumerate(HEAD):
        head_reads[k].wait()
        segment(sum(HEAD[:k]), units)

    def early_step(i, _):
        for k, copies in enumerate(step_reads):
            for copy in copies:
                pl.when(i == k)(copy.wait)
        segment(sum(HEAD), LOOP_UNITS, i)

    lax.fori_loop(0, EARLY_STEPS, early_step, None)
    lax.fori_loop(EARLY_STEPS, LOOP_STEPS, lambda i, _: segment(sum(HEAD), LOOP_UNITS, i, True), None)
    pltpu.make_async_copy(o_ref, o_hbm, sems.at[0]).wait()


@jax.jit
def pallas_standalone__layernorm_linear__sampling_kernel(
    x: jax.Array,
    g: jax.Array,
    b: jax.Array,
    w: jax.Array,
):
    assert x.shape == (L, S, D) and w.shape == (D, D)
    hbm = pl.BlockSpec(memory_space=pl.ANY)
    out = pl.pallas_call(
        _kernel,
        in_specs=[hbm] * 4,
        out_specs=hbm,
        out_shape=jax.ShapeDtypeStruct((2 * S, HALF, L), bf16),
        scratch_shapes=[
            pltpu.VMEM((3 * (LATE_SLAB + 1), THIRD, L), bf16),
            pltpu.VMEM((3 * (S - LATE_SLAB) + 1, THIRD, L), bf16),
            pltpu.VMEM((2 * S, HALF, L), bf16),
            pltpu.VMEM((_X_ROWS, 128), bf16),
            pltpu.VMEM((_X_ROWS, 128), bf16),
            pltpu.VMEM((D, 128), f32),
            pltpu.VMEM((D, D), bf16),
            pltpu.VMEM((5, D, 128), bf16),
            pltpu.VMEM((-(-len(_W_TILE) // 4) * 4, QUARTER, 128), bf16),
            pltpu.VMEM((D,), bf16),
            pltpu.VMEM((D,), bf16),
            pltpu.SMEM((4,), jnp.int32),
            pltpu.SemaphoreType.DMA((16,)),
        ],
        compiler_params=pltpu.CompilerParams(
            vmem_limit_bytes=110 * 2**20,
            disable_bounds_checks=True,
            disable_semaphore_checks=True,
        ),
        name="layernorm_linear",
    )(jnp.transpose(x, (1, 2, 0)).reshape(3 * S, THIRD, L), g, b, w)
    return jnp.transpose(out.reshape(S, D, L), (2, 0, 1))
```
